```python
import os as _os
_os.environ.setdefault("JAX_PLATFORMS", "cpu")
import jax
import jax.numpy as jnp

def _softmax(x, axis=-1):
    return jax.nn.softmax(x, axis=axis)
def _gelu(x):
    return jax.nn.gelu(x, approximate=True)
def _silu(x):
    return jax.nn.silu(x)
def _sigmoid(x):
    return jax.nn.sigmoid(x)
def _layernorm(x, axis=-1, eps=1e-5):
    m = jnp.mean(x, axis=axis, keepdims=True)
    v = jnp.var(x, axis=axis, keepdims=True)
    return (x - m) / jnp.sqrt(v + eps)
def _scatter_add(tgt, idx, src, axis=0):
    return tgt.at[idx].add(src)
def _segment_sum(src, seg, n):
    return jax.ops.segment_sum(src, seg, n)
class _Rng:
    def __init__(self, key):
        self._k = key
    def _next(self):
        self._k, sub = jax.random.split(self._k)
        return sub
    def normal(self, shape):
        return jax.random.normal(self._next(), shape, dtype=jnp.bfloat16)
    def randint(self, lo, hi, shape):
        return jax.random.randint(self._next(), shape, lo, hi, dtype=jnp.int32)
    def uniform(self, shape, lo=0.0, hi=1.0):
        return jax.random.uniform(self._next(), shape, jnp.bfloat16, lo, hi)
    def permutation(self, n):
        return jax.random.permutation(self._next(), n)


kernel_name = 'parallel_sum__ssm_conv_s4__mixer_channel_mlp__prompt'

def setup_inputs():
    _rng = _Rng(jax.random.key(int.from_bytes(__import__("os").urandom(4), "little")))
    _w = (lambda a: (lambda t: t.astype(jnp.bfloat16) if jnp.issubdtype(t.dtype, jnp.floating) else t)(jnp.asarray(a)))
    def _A_setup():
        B, L, D, N = 1, 2048, 512, 128
        A_re = -jnp.exp((lambda *s: _rng.normal(s) * 0.1)(D, N))
        A_im = jnp.pi * (lambda *s: _rng.normal(s) * 0.1)(D, N)
        B_re = (lambda *s: _rng.normal(s) * 0.1)(D, N)
        B_im = (lambda *s: _rng.normal(s) * 0.1)(D, N)
        C_re = (lambda *s: _rng.normal(s) * 0.1)(D, N)
        C_im = (lambda *s: _rng.normal(s) * 0.1)(D, N)
        log_dt = (lambda *s: _rng.normal(s) * 0.1)(D) * 0.5 - 4.0
        Dskip = (lambda *s: _rng.normal(s) * 0.05)(D)
        return {
            "u": _w((lambda *s: _rng.normal(s) * 0.05)(B, L, D)),
            "A_re": _w(A_re),
            "A_im": _w(A_im),
            "B_re": _w(B_re),
            "B_im": _w(B_im),
            "C_re": _w(C_re),
            "C_im": _w(C_im),
            "log_dt": _w(log_dt),
            "Dskip": _w(Dskip),
        }
    _A_in = _A_setup()

    def _B_setup():
        B, S, D, F = 1, 2048, 512, 1792
        return {
            "x": _w((lambda *s: _rng.normal(s) * 0.05)(B, S, D)),
            "w1": _w((lambda *s: _rng.normal(s) * 0.2)(D, F) * (D ** -0.5)),
            "b1": _w((lambda *s: _rng.normal(s) * 0.2)(F)),
            "w2": _w((lambda *s: _rng.normal(s) * 0.2)(F, D) * (F ** -0.5)),
            "b2": _w((lambda *s: _rng.normal(s) * 0.05)(D)),
        }
    _B_in = _B_setup()

    return {
        "A_u": _A_in["u"],
        "A_A_re": _A_in["A_re"],
        "A_A_im": _A_in["A_im"],
        "A_B_re": _A_in["B_re"],
        "A_B_im": _A_in["B_im"],
        "A_C_re": _A_in["C_re"],
        "A_C_im": _A_in["C_im"],
        "A_log_dt": _A_in["log_dt"],
        "A_Dskip": _A_in["Dskip"],
        "B_x": _B_in["x"],
        "B_w1": _B_in["w1"],
        "B_b1": _B_in["b1"],
        "B_w2": _B_in["w2"],
        "B_b2": _B_in["b2"],
    }

def reference(A_u, A_A_re, A_A_im, A_B_re, A_B_im, A_C_re, A_C_im, A_log_dt, A_Dskip, B_x, B_w1, B_b1, B_w2, B_b2):
    def _A_ref(u, A_re, A_im, B_re, B_im, C_re, C_im, log_dt, Dskip):
        Bsz, L, D = u.shape
        dt = jnp.exp(log_dt)[:, None]
        A = A_re + 1j * A_im
        Bc = B_re + 1j * B_im
        Cc = C_re + 1j * C_im
        logdA = dt * A
        dB = dt * Bc
        l = (lambda x, dt: x.astype(dt))(jnp.arange(L), A_re.dtype)
        P = jnp.exp(logdA[:, :, None] * l[None, None, :])
        K = jnp.einsum("dn,dnl,dn->dl", Cc, P, dB).real
        L2 = 2 * L
        Kp = jnp.pad(K, ((0, 0), (0, L)))
        up = (lambda x, *d: x.transpose(*d))(u, 0, 2, 1)
        up = jnp.pad(up, ((0, 0), (0, 0), (0, L)))
        Kf = (lambda x, axes=(-2,-1): jnp.fft.rfft2(x.astype(jnp.float32), axes=axes))(Kp[:, None, :], axes=(-2, -1))
        Uf = (lambda x, axes=(-2,-1): jnp.fft.rfft2(x.astype(jnp.float32), axes=axes))(up[:, :, None, :], axes=(-2, -1))
        Yf = Uf * Kf[None, :, :, :]
        y = (lambda x, s, axes=(-2,-1): jnp.fft.irfft2(x, s=s, axes=axes).astype(jnp.bfloat16))(Yf, (1, L2), axes=(-2, -1))[:, :, 0, :L]
        y = (lambda x, *d: x.transpose(*d))(y, 0, 2, 1) + u * Dskip[None, None, :]
        return y

    def _B_ref(x, w1, b1, w2, b2):
        y = _layernorm(x, axis=-1)
        h = _gelu(jnp.einsum("bsd,df->bsf", y, w1) + b1)
        return jnp.einsum("bsf,fd->bsd", h, w2) + b2

    x = A_u
    xn = _layernorm(x, axis=-1)
    return x + _A_ref(xn, A_A_re, A_A_im, A_B_re, A_B_im, A_C_re, A_C_im, A_log_dt, A_Dskip) + _B_ref(xn, B_w1, B_b1, B_w2, B_b2)
```

```python
import functools
import numpy as np
import jax
import jax.numpy as jnp
import jax.experimental.pallas as pl
import jax.experimental.pallas.tpu as pltpu

L, D, N, FF, T = 2048, 512, 128, 1792, 128
NCH = L // T
f32, bf16 = jnp.float32, jnp.bfloat16

def _bf16_round_int(l):
    out = np.zeros_like(l)
    for i, v in enumerate(l):
        v = int(v)
        if v < 256:
            out[i] = v
        else:
            e = v.bit_length() - 8
            s = 1 << e
            q, r = divmod(v, s)
            if r * 2 > s or (r * 2 == s and (q & 1)):
                q += 1
            out[i] = q * s
    return out

_l = np.arange(L)
_r = _bf16_round_int(_l)
_R = np.unique(_r)
_idx = np.searchsorted(_R, _r)
NR = 648
_off = [int(np.searchsorted(_R, 128 * m)) for m in range(NCH)]
_wid = []
for m in range(NCH):
    hi = int(_idx[128 * m:128 * (m + 1)].max())
    _wid.append(((hi - _off[m]) // 8 + 1) * 8)

_c = np.arange(T)
_f = np.arange(128)
_Fp = np.zeros((256, T))
_Fp[:128] = np.cos(2 * np.pi * _f[:, None] * _c[None, :] / 256)
_Fp[128] = np.cos(np.pi * _c)
_Fp[129:] = -np.sin(2 * np.pi * _f[1:, None] * _c[None, :] / 256)
PHIW = 136
_PhiAll = np.zeros((NCH, 256, PHIW))
for m in range(NCH):
    for c in range(T):
        _PhiAll[m, :, _idx[128 * m + c] - _off[m]] += _Fp[:, c]
_p = np.arange(256)
_Gp = np.zeros((256, 256))
_Gp[:, 0] = 1.0 / 256
_Gp[:, 1:128] = 2 * np.cos(2 * np.pi * _p[:, None] * _f[None, 1:] / 256) / 256
_Gp[:, 128] = np.cos(np.pi * _p) / 256
_Gp[:, 129:] = -2 * np.sin(2 * np.pi * _p[:, None] * _f[None, 1:] / 256) / 256

SEGS = [(1, 0, 16), (2, 256, 8), (4, 512, 8), (8, 1024, 8)]


def _cmul(ar, ai, br, bi):
    return ar * br - ai * bi, ar * bi + ai * br


def _ln_bf16(x32):
    m = jnp.mean(x32, axis=-1, keepdims=True)
    v = jnp.mean((x32 - m) * (x32 - m), axis=-1, keepdims=True)
    mb = m.astype(bf16).astype(f32)
    db = (x32 - mb).astype(bf16).astype(f32)
    vb = v.astype(bf16).astype(f32)
    den = jnp.sqrt((vb + 1e-5).astype(bf16).astype(f32)).astype(bf16).astype(f32)
    return (db / den).astype(bf16)


class _KG:
    def __init__(self, pt_ref, dt_ref, p_ref, row, ds_):
        self.pt_ref, self.dt_ref, self.p_ref, self.row, self.ds_ = pt_ref, dt_ref, p_ref, row, ds_
        self.pw = None
    def init(self):
        dtb = self.dt_ref[:, self.ds_]
        ld = lambda t: self.pt_ref[t, pl.ds(self.row, 8), self.ds_]
        ar = dtb * ld(0); ai = dtb * ld(1)
        er = jnp.exp(ar)
        z = (er * jnp.cos(ai), er * jnp.sin(ai))
        dbr = dtb * ld(2); dbi = dtb * ld(3)
        self.c = _cmul(ld(4), ld(5), dbr, dbi)
        self.pw = {0: (jnp.ones_like(er), jnp.zeros_like(er)), 1: z}
    def getp(self, k):
        if self.pw is None:
            self.init()
        pw = self.pw
        if k not in pw:
            h = k // 2
            a = self.getp(h); b_ = self.getp(k - h)
            pw[k] = _cmul(a[0], a[1], b_[0], b_[1])
        return pw[k]
    def part(self, s, base, q, k0):
        pr, pi = self.getp(base + 16 * s * q)
        cr, ci = self.c
        xr, xi = _cmul(cr, ci, pr, pi)
        for j in range(16):
            fr, fi = self.getp(s * j)
            self.p_ref[pl.ds(8 * (k0 + j), 8), self.ds_] += xr * fr - xi * fi
    def lastp(self):
        pr, pi = self.getp(2048)
        cr, ci = self.c
        xr, _ = _cmul(cr, ci, pr, pi)
        self.p_ref[pl.ds(8 * 640, 8), self.ds_] += xr


def kgen_parts(pt_ref, dt_ref, p_ref, g):
    row = pl.multiple_of(8 * g, 8)
    out = []
    for b in range(D // 128):
        kg = _KG(pt_ref, dt_ref, p_ref, row, slice(128 * b, 128 * b + 128))
        k0 = 0
        for (s, base, nq) in SEGS:
            for q in range(nq):
                out.append(functools.partial(kg.part, s, base, q, k0))
                k0 += 16
        out.append(kg.lastp)
    return out

FB = 256
TM = 256
NS1 = L // TM
CPS = TM // T
GPS = (N // 8) // NS1

def kernel(x_ref, are_ref, aim_ref, bre_ref, bim_ref, cre_ref, cim_ref, ldt_ref, dsk_ref,
           w1_ref, b1_ref, w2_ref, b2_ref, fp_ref, phi_ref, g_ref,
           o_ref,
           p_ref, pt_ref, dt_ref, khat_ref, uhat_ref, z_ref, xs_ref, xn_ref, mo_ref):
    i = pl.program_id(0)

    @pl.when(i == 0)
    def _():
        dt_ref[...] = jnp.exp(ldt_ref[...].astype(f32)).astype(bf16).astype(f32)
        for t, r in enumerate((are_ref, aim_ref, bre_ref, bim_ref, cre_ref, cim_ref)):
            pt_ref[t] = jnp.transpose(r[...].astype(f32))
        p_ref[...] = jnp.zeros_like(p_ref)

    @pl.when(i < NS1)
    def _phase1():
        parts = []
        for gg in range(GPS):
            parts += kgen_parts(pt_ref, dt_ref, p_ref, i * GPS + gg)
        x = x_ref[...]
        r0 = pl.multiple_of(i * TM, TM)
        xs_ref[pl.ds(r0, TM), :] = x
        xn = _ln_bf16(x.astype(f32))
        xn_ref[pl.ds(r0, TM), :] = xn
        for cc in range(CPS):
            uhat_ref[i * CPS + cc] = jnp.dot(fp_ref[...], xn[cc * T:(cc + 1) * T], preferred_element_type=f32)
        y2 = _ln_bf16(xn.astype(f32))
        nb = FF // FB
        per = -(-len(parts) // nb)
        acc = None
        for fb in range(nb):
            cs = slice(fb * FB, fb * FB + FB)
            h = jnp.dot(y2, w1_ref[:, cs], preferred_element_type=f32) + b1_ref[:, cs].astype(f32)
            h = jax.nn.gelu(h, approximate=True).astype(bf16)
            pp = jnp.dot(h, w2_ref[cs, :], preferred_element_type=f32)
            acc = pp if acc is None else acc + pp
            for pt in parts[fb * per:(fb + 1) * per]:
                pt()
        mo_ref[pl.ds(r0, TM), :] = (acc.astype(bf16).astype(f32) + b2_ref[...].astype(f32)).astype(bf16)

    @pl.when(i == NS1)
    def _phase2():
        for m in range(NCH):
            pp = p_ref[pl.ds(8 * _off[m], 8 * _wid[m]), :].reshape(_wid[m], 8, D)
            kb = jnp.sum(pp, axis=1).astype(bf16)
            khat_ref[m] = jnp.dot(phi_ref[m, :, :_wid[m]], kb, preferred_element_type=f32)
        def tile(t, carry):
            r0 = pl.multiple_of(t * 8, 8)
            for c in range(NCH):
                zr = zi = None
                for j in range(c + 1):
                    ur = uhat_ref[j, pl.ds(r0, 8), :]; ui = uhat_ref[j, pl.ds(128 + r0, 8), :]
                    kr = khat_ref[c - j, pl.ds(r0, 8), :]; ki = khat_ref[c - j, pl.ds(128 + r0, 8), :]
                    tr = ur * kr - ui * ki; ti = ur * ki + ui * kr
                    if zr is None:
                        zr, zi = tr, ti
                    else:
                        zr, zi = zr + tr, zi + ti
                z_ref[c, pl.ds(r0, 8), :] = zr
                z_ref[c, pl.ds(128 + r0, 8), :] = zi
            return carry
        jax.lax.fori_loop(0, 16, tile, 0)
        for c in range(NCH):
            for r in (0, 128):
                acc = None
                for j in range(c + 1):
                    v = uhat_ref[j, pl.ds(r, 1), :] * khat_ref[c - j, pl.ds(r, 1), :]
                    acc = v if acc is None else acc + v
                z_ref[c, pl.ds(r, 1), :] = acc
        dsk = dsk_ref[...].astype(f32)
        for c in range(NCH):
            y = jnp.dot(g_ref[0], z_ref[c].astype(bf16), preferred_element_type=f32)
            if c > 0:
                y = y + jnp.dot(g_ref[1], z_ref[c - 1].astype(bf16), preferred_element_type=f32)
            rs = slice(c * T, (c + 1) * T)
            yb = y.astype(bf16).astype(f32)
            xnf = xn_ref[rs, :].astype(f32)
            a_out = (yb + (xnf * dsk).astype(bf16).astype(f32)).astype(bf16).astype(f32)
            o_ref[rs, :] = ((xs_ref[rs, :].astype(f32) + a_out).astype(bf16).astype(f32) + mo_ref[rs, :].astype(f32)).astype(o_ref.dtype)


@jax.jit
def pallas_parallel_sum__ssm_conv_s4__mixer_channel_mlp__prompt_kernel(A_u, A_A_re, A_A_im, A_B_re, A_B_im, A_C_re, A_C_im, A_log_dt, A_Dskip, B_x, B_w1, B_b1, B_w2, B_b2):
    x = A_u.reshape(L, D)
    full = lambda shp: pl.BlockSpec(shp, lambda i: tuple(0 for _ in shp))
    fp = jnp.asarray(_Fp, bf16); phi = jnp.asarray(_PhiAll, bf16)
    g = jnp.asarray(np.stack([_Gp[:128], _Gp[128:]]), bf16)
    out = pl.pallas_call(
        kernel, grid=(NS1 + 1,),
        in_specs=[pl.BlockSpec((TM, D), lambda i: (jnp.minimum(i, NS1 - 1), 0))] + [full((D, N))] * 6 + [full((1, D)), full((1, D)),
                  full((D, FF)), full((1, FF)), full((FF, D)), full((1, D)),
                  full((256, T)), full((NCH, 256, PHIW)), full((2, 128, 256))],
        out_specs=full((L, D)),
        out_shape=jax.ShapeDtypeStruct((L, D), bf16),
        scratch_shapes=[pltpu.VMEM((NR * 8, D), f32), pltpu.VMEM((6, N, D), f32), pltpu.VMEM((1, D), f32),
                        pltpu.VMEM((NCH, 256, D), f32), pltpu.VMEM((NCH, 256, D), f32), pltpu.VMEM((NCH, 256, D), f32),
                        pltpu.VMEM((L, D), bf16), pltpu.VMEM((L, D), bf16), pltpu.VMEM((L, D), bf16)],
        compiler_params=pltpu.CompilerParams(dimension_semantics=("arbitrary",), vmem_limit_bytes=110 * 1024 * 1024),
    )(x, A_A_re, A_A_im, A_B_re, A_B_im, A_C_re, A_C_im, A_log_dt.reshape(1, D), A_Dskip.reshape(1, D),
      B_w1, B_b1.reshape(1, FF), B_w2, B_b2.reshape(1, D), fp, phi, g)
    return out.reshape(1, L, D)
```
